```python
import jax
import jax.numpy as jnp

def _softmax(x, axis=-1):
    return jax.nn.softmax(x, axis=axis)
def _gelu(x):
    return jax.nn.gelu(x, approximate=True)
def _silu(x):
    return jax.nn.silu(x)
def _sigmoid(x):
    return jax.nn.sigmoid(x)
def _layernorm(x, axis=-1, eps=1e-5):
    m = jnp.mean(x, axis=axis, keepdims=True)
    v = jnp.var(x, axis=axis, keepdims=True)
    return (x - m) / jnp.sqrt(v + eps)
def _scatter_add(tgt, idx, src, axis=0):
    return tgt.at[idx].add(src)
def _segment_sum(src, seg, n):
    return jax.ops.segment_sum(src, seg, n)
class _Rng:
    def __init__(self, key):
        self._k = key
    def _next(self):
        self._k, sub = jax.random.split(self._k)
        return sub
    def normal(self, shape):
        return jax.random.normal(self._next(), shape, dtype=jnp.bfloat16)
    def randint(self, lo, hi, shape):
        return jax.random.randint(self._next(), shape, lo, hi, dtype=jnp.int32)
    def uniform(self, shape, lo=0.0, hi=1.0):
        return jax.random.uniform(self._next(), shape, jnp.bfloat16, lo, hi)
    def permutation(self, n):
        return jax.random.permutation(self._next(), n)


kernel_name = 'gated_mix__sliding_local_dilated__compressed_kv_cla__prompt'

def setup_inputs():
    _rng = _Rng(jax.random.key(int.from_bytes(__import__("os").urandom(4), "little")))
    _w = (lambda a: (lambda t: t.astype(jnp.bfloat16) if jnp.issubdtype(t.dtype, jnp.floating) else t)(jnp.asarray(a)))
    def _A_setup():
        B, S, D = 1, 2048, 576
        return {
            "x": _w((lambda *s: _rng.normal(s) * 0.05)(B, S, D)),
            "wqkv": _w((lambda *s: _rng.normal(s) * 0.05)(D, 3 * D)),
            "wo": _w((lambda *s: _rng.normal(s) * 0.05)(D, D)),
        }
    _A_in = _A_setup()

    def _B_setup():
        B, H, Sq, Sk, D, M = 1, 32, 2048, 2048, 128, 576
        Dc = 4 * D
        return {
            "x": _w((lambda *s: _rng.normal(s) * 0.05)(B, Sq, M)),
            "c_kv": _w((lambda *s: _rng.normal(s) * 0.05)(B, Sk, Dc)),
            "w_q": _w((lambda *s: _rng.normal(s) * 0.05)(M, H, D) * (M ** -0.5)),
            "w_uk": _w((lambda *s: _rng.normal(s) * 0.05)(Dc, H, D) * (Dc ** -0.5)),
            "w_uv": _w((lambda *s: _rng.normal(s) * 0.05)(Dc, H, D) * (Dc ** -0.5)),
            "w_o": _w((lambda *s: _rng.normal(s) * 0.05)(H, D, M) * ((H * D) ** -0.5)),
        }
    _B_in = _B_setup()

    return {
        "A_x": _A_in["x"],
        "A_wqkv": _A_in["wqkv"],
        "A_wo": _A_in["wo"],
        "B_x": _B_in["x"],
        "B_c_kv": _B_in["c_kv"],
        "B_w_q": _B_in["w_q"],
        "B_w_uk": _B_in["w_uk"],
        "B_w_uv": _B_in["w_uv"],
        "B_w_o": _B_in["w_o"],
        "gate_w": _w((lambda *s: _rng.normal(s) * 0.05)(576)),
    }

def reference(A_x, A_wqkv, A_wo, B_x, B_c_kv, B_w_q, B_w_uk, B_w_uv, B_w_o, gate_w):
    def _A_ref(x, wqkv, wo):
        B, S, D = x.shape
        H = 32; Dh = D // H
        W, dil = 8, 2
        qkv = (lambda x, *d: x.transpose(*d))((x @ wqkv).reshape(B, S, 3, H, Dh), 2, 0, 3, 1, 4)
        q, k, v = qkv[0], qkv[1], qkv[2]
        scale = Dh ** -0.5
        pos = jnp.arange(S)
        off = jnp.arange(W) * dil
        idx = pos[:, None] - off[None, :]
        mask = idx >= 0
        idx_c = jnp.where(mask, idx, 0).reshape(-1)
        kg = k[:, :, idx_c, :].reshape(B, H, S, W, Dh)
        vg = v[:, :, idx_c, :].reshape(B, H, S, W, Dh)
        logits = jnp.einsum("bhsd,bhswd->bhsw", q, kg) * scale
        logits = jnp.where(mask[None, None, :, :], logits, -1e9)
        attn = _softmax(logits, axis=-1)
        o = jnp.einsum("bhsw,bhswd->bhsd", attn, vg)
        return (lambda x, *d: x.transpose(*d))(o, 0, 2, 1, 3).reshape(B, S, D) @ wo

    def _B_ref(x, c_kv, w_q, w_uk, w_uv, w_o):
        B, Sq, M = x.shape[0], x.shape[1], x.shape[2]
        Sk = c_kv.shape[1]
        H, D = w_q.shape[1], w_q.shape[2]
        q = jnp.einsum("bqm,mhd->bhqd", x, w_q)
        k = jnp.einsum("bkc,chd->bhkd", c_kv, w_uk)
        v = jnp.einsum("bkc,chd->bhkd", c_kv, w_uv)
        scores = jnp.einsum("bhqd,bhkd->bhqk", q, k) * (D ** -0.5)
        off = Sk - Sq
        qi = jnp.arange(Sq)[:, None]
        kj = jnp.arange(Sk)[None, :]
        cmask = kj <= (qi + off)
        scores = jnp.where(cmask[None, None], scores, -1e9)
        p = _softmax(scores, axis=-1)
        ctx = jnp.einsum("bhqk,bhkd->bhqd", p, v)
        return jnp.einsum("bhqd,hdm->bqm", ctx, w_o)

    x = A_x
    g = _sigmoid((x * gate_w).sum(-1, keepdims=True))
    a = _A_ref(x, A_wqkv, A_wo)
    b = _B_ref(x, B_c_kv, B_w_q, B_w_uk, B_w_uv, B_w_o)
    return g * a + (1 - g) * b
```

```python
import functools
import jax
import jax.numpy as jnp
import numpy as np
import jax.experimental.pallas as pl
import jax.experimental.pallas.tpu as pltpu

S, M, H, D, DC = 2048, 576, 32, 128, 512
DH = 18
MP = 640
BQ = 256
CH = 256
LOG2E = 1.4426950408889634
F32, BF16 = jnp.float32, jnp.bfloat16
NT = (((1,), (1,)), ((), ()))


def _pair(ref, j, rows):
    u = ref.bitcast(jnp.uint32)[:, j % 8, :]
    lo = pltpu.bitcast(u << 16, F32).astype(BF16)
    hi = pltpu.bitcast(u & jnp.uint32(0xFFFF0000), F32).astype(BF16)
    return jnp.concatenate([lo, hi], axis=1)


def _kernel(x_ref, wqkv_ref, wo_ref, c_ref, wq_ref, wuk_ref, wuv_ref, wob_ref, gw_ref,
            o_ref, acc_ref, g_ref, q_s, k_s, v_s, ctx_s, wt_s, wp_s, wop_s, ka_s, va_s):
    j = pl.program_id(0)

    @pl.when(j == 0)
    def _prologue():
        for t in range(5):
            blk = wqkv_ref[t * 128:min(M, t * 128 + 128), :].astype(F32)
            if t == 4:
                blk = jnp.concatenate([blk, jnp.zeros_like(blk)], axis=0)
            wt_s[t] = blk.T
        for p in range(3):
            for d in range(DH):
                for t in range(5):
                    wp_s[p * MP + d * 32:p * MP + d * 32 + 32, t * 128:t * 128 + 128] = wt_s[t, pl.ds(p * M + d, 32, stride=DH), :].astype(BF16)
            wp_s[p * MP + M:(p + 1) * MP, :] = jnp.zeros((MP - M, MP), BF16)
        for t in range(5):
            cw = min(128, M - t * 128)
            wt_s[t, 0:M, 0:cw] = wo_ref[:, t * 128:t * 128 + cw].astype(F32)
        for d in range(DH):
            for t in range(5):
                wop_s[d * 32:d * 32 + 32, t * 128:t * 128 + 128] = wt_s[t, pl.ds(d, 32, stride=DH), :].astype(BF16)
        wop_s[M:MP, :] = jnp.zeros((MP - M, MP), BF16)
        ka_s[0:16, :] = jnp.zeros((16, MP), F32)
        va_s[0:16, :] = jnp.zeros((16, MP), F32)

        def chunk(c, carry):
            r0 = pl.multiple_of(c * CH, CH)
            xc = x_ref[pl.ds(r0, CH), :]
            qkv = jax.lax.dot_general(xc, wp_s[:, 0:M], NT, preferred_element_type=F32)
            ka_s[pl.ds(r0 + 16, CH), :] = qkv[:, MP:2 * MP]
            va_s[pl.ds(r0 + 16, CH), :] = qkv[:, 2 * MP:]
            q = qkv[:, :MP] * (DH ** -0.5 * LOG2E)
            gl = jnp.sum(xc.astype(F32) * gw_ref[...].astype(F32), axis=-1, keepdims=True)
            g = jax.nn.sigmoid(jnp.broadcast_to(gl, (CH, 128)))
            g_ref[pl.ds(r0, CH), :] = 1.0 - g
            kk = ka_s[pl.ds(r0, CH + 16), :]
            vv = va_s[pl.ds(r0, CH + 16), :]
            row = r0 + jax.lax.broadcasted_iota(jnp.int32, (CH, 128), 0)
            lg = []
            for w in range(8):
                pr = q * kk[16 - 2 * w:16 - 2 * w + CH, :]
                t = pr[:, 0:128] + pr[:, 128:256] + pr[:, 256:384] + pr[:, 384:512] + pr[:, 512:640]
                t = t + pltpu.roll(t, 64, 1)
                t = t + pltpu.roll(t, 32, 1)
                if w > 0:
                    t = jnp.where(row >= 2 * w, t, -1e9)
                lg.append(t)
            m = functools.reduce(jnp.maximum, lg)
            e = [jnp.exp2(t - m) for t in lg]
            inv = g / functools.reduce(jnp.add, e)
            o = None
            for w in range(8):
                a = e[w] * inv
                t = jnp.concatenate([a] * 5, axis=1) * vv[16 - 2 * w:16 - 2 * w + CH, :]
                o = t if o is None else o + t
            acc_ref[pl.ds(r0, CH), :] = jnp.dot(o.astype(BF16), wop_s[:, 0:M], preferred_element_type=F32)
            return carry

        jax.lax.fori_loop(0, S // CH, chunk, 0)

    wq = _pair(wq_ref, j, M)
    wk = _pair(wuk_ref, j, DC)
    wv = _pair(wuv_ref, j, DC)
    for r in range(0, S, 512):
        q = jnp.dot(x_ref[r:r + 512, :], wq, preferred_element_type=F32) * (D ** -0.5 * LOG2E)
        k = jnp.dot(c_ref[r:r + 512, :], wk, preferred_element_type=F32)
        v = jnp.dot(c_ref[r:r + 512, :], wv, preferred_element_type=F32)
        q_s[r:r + 512, :] = q.astype(BF16)
        k_s[r:r + 512, :] = k.astype(BF16)
        v_s[r:r + 512, :] = v.astype(BF16)

    tri = (jax.lax.broadcasted_iota(jnp.int32, (BQ, BQ), 1) <= jax.lax.broadcasted_iota(jnp.int32, (BQ, BQ), 0))
    wob = wob_ref[...]
    for i in range(S // BQ):
        r0, r1 = i * BQ, (i + 1) * BQ
        for hh in range(2):
            cs = slice(hh * 128, hh * 128 + 128)
            q = q_s[r0:r1, cs]
            sd = jax.lax.dot_general(q, k_s[r0:r1, cs], NT, preferred_element_type=F32)
            sd = jnp.where(tri, sd, -1e9)
            m = jnp.max(sd, axis=-1, keepdims=True)
            if i > 0:
                s = jax.lax.dot_general(q, k_s[0:r0, cs], NT, preferred_element_type=F32)
                m = jnp.maximum(m, jnp.max(s, axis=-1, keepdims=True))
            pd = jnp.exp2(sd - m)
            l = jnp.sum(pd, axis=-1, keepdims=True)
            ctx = jnp.dot(pd.astype(BF16), v_s[r0:r1, cs], preferred_element_type=F32)
            if i > 0:
                p = jnp.exp2(s - m)
                l = l + jnp.sum(p, axis=-1, keepdims=True)
                ctx = ctx + jnp.dot(p.astype(BF16), v_s[0:r0, cs], preferred_element_type=F32)
            ctx_s[r0:r1, cs] = (ctx * (g_ref[r0:r1, :] / l)).astype(BF16)
        acc_ref[r0:r1, :] += jnp.dot(ctx_s[r0:r1, :], wob, preferred_element_type=F32)

    @pl.when(j == H // 2 - 1)
    def _():
        o_ref[...] = acc_ref[...].astype(o_ref.dtype)


@jax.jit
def pallas_gated_mix__sliding_local_dilated__compressed_kv_cla__prompt_kernel(
    A_x, A_wqkv, A_wo, B_x, B_c_kv, B_w_q, B_w_uk, B_w_uv, B_w_o, gate_w,
):
    del B_x
    full = lambda shape: pl.BlockSpec(shape, lambda j: (0, 0), pipeline_mode=pl.Buffered(1))
    hs = lambda r: pl.BlockSpec((r, 16, D), lambda j: (0, j // 8, 0))
    out = pl.pallas_call(
        _kernel,
        grid=(H // 2,),
        in_specs=[
            full((S, M)), full((M, 3 * M)), full((M, M)), full((S, DC)),
            hs(M), hs(DC), hs(DC),
            pl.BlockSpec((2 * D, M), lambda j: (j, 0)),
            full((1, M)),
        ],
        out_specs=pl.BlockSpec((S, M), lambda j: (0, 0)),
        out_shape=jax.ShapeDtypeStruct((S, M), BF16),
        scratch_shapes=[
            pltpu.VMEM((S, M), F32), pltpu.VMEM((S, 128), F32),
            pltpu.VMEM((S, 256), BF16), pltpu.VMEM((S, 256), BF16), pltpu.VMEM((S, 256), BF16), pltpu.VMEM((S, 256), BF16),
            pltpu.VMEM((5, 3 * M, 128), F32), pltpu.VMEM((3 * MP, MP), BF16), pltpu.VMEM((MP, MP), BF16),
            pltpu.VMEM((S + 16, MP), F32), pltpu.VMEM((S + 16, MP), F32),
        ],
        compiler_params=pltpu.CompilerParams(dimension_semantics=("arbitrary",), vmem_limit_bytes=110 * 1024 * 1024),
    )(A_x.reshape(S, M), A_wqkv, A_wo, B_c_kv.reshape(S, DC), B_w_q,
      B_w_uk, B_w_uv, B_w_o.reshape(H * D, M), gate_w.reshape(1, M))
    return out.reshape(1, S, M)
```

```python
import functools
import jax
import jax.numpy as jnp
import jax.experimental.pallas as pl
import jax.experimental.pallas.tpu as pltpu

S, M, H, D, DC = 2048, 576, 32, 128, 512
DH = 18
MP = 640
BQ = 256
NQ = S // BQ
CH = 512
STEPS = H // 2
AC = S // STEPS
SC = AC // 4
LOG2E = 1.4426950408889634
F32, BF16, U32 = jnp.float32, jnp.bfloat16, jnp.uint32
NT = (((1,), (1,)), ((), ()))


def _nt(a, b):
    return jax.lax.dot_general(a, b, NT, preferred_element_type=F32)


def _nn(a, b):
    return jnp.dot(a, b, preferred_element_type=F32)


def _recip(l):
    r = pl.reciprocal(l, approx=True)
    return r * (2.0 - l * r)


def _pair(ref, j, rows):
    u = ref[pl.ds(j, rows, stride=STEPS), :]
    lo = pltpu.bitcast(u << 16, F32).astype(BF16)
    hi = pltpu.bitcast(u & jnp.uint32(0xFFFF0000), F32).astype(BF16)
    return jnp.concatenate([lo, hi], axis=1)


def _kernel(xt_hbm, wqkv_hbm, wo_hbm, c_hbm, wq_hbm, wuk_hbm, wuv_hbm, wob_ref, gw_ref,
            o_hbm, acc_ref, a_s, g_ref, q_s, k_s, v_s, ctx_s, wt_s, wp_s, wop_s, wopt_s,
            qa_s, ka_s, va_s, x_ref, c_ref, wq_s, wk_s, wv_s, xt_ref, wqkv_ref, wo_ref, sems):
    j = pl.program_id(0)

    @pl.when(j == 0)
    def _prologue():
        rows = [slice(t * 128, min(M, t * 128 + 128)) for t in range(5)]
        wcp = [pltpu.make_async_copy(wqkv_hbm.at[r], wqkv_ref.at[r], sems.at[5 + t]) for t, r in enumerate(rows)]
        xcp = lambda c, r0: pltpu.make_async_copy(
            xt_hbm.at[:, pl.ds(r0, CH)], xt_ref.at[:, pl.ds(r0, CH)], sems.at[10 + c])
        ocp = pltpu.make_async_copy(wo_hbm, wo_ref, sems.at[4])
        for c in wcp:
            c.start()
        xcp(0, 0).start()
        copies = [
            pltpu.make_async_copy(wq_hbm.bitcast(U32), wq_s, sems.at[0]),
            pltpu.make_async_copy(c_hbm, c_ref, sems.at[1]),
            pltpu.make_async_copy(wuk_hbm.bitcast(U32), wk_s, sems.at[2]),
            pltpu.make_async_copy(wuv_hbm.bitcast(U32), wv_s, sems.at[3]),
        ]
        for t in range(5):
            wcp[t].wait()
            blk = wqkv_ref[t * 128:min(M, t * 128 + 128), :].astype(F32)
            if t == 4:
                blk = jnp.concatenate([blk, jnp.zeros_like(blk)], axis=0)
            wt_s[t] = blk.T
        for c in range(1, S // CH):
            xcp(c, c * CH).start()
        ocp.start()
        for c in copies:
            c.start()
        for p in range(3):
            for d in range(DH):
                for t in range(5):
                    wp_s[p * MP + d * 32:p * MP + d * 32 + 32, t * 128:t * 128 + 128] = (
                        wt_s[t, pl.ds(p * M + d, 32, stride=DH), :].astype(BF16))
            wp_s[p * MP + M:(p + 1) * MP, :] = jnp.zeros((MP - M, MP), BF16)
        ka_s[0:16, :] = jnp.zeros((16, MP), F32)
        va_s[0:16, :] = jnp.zeros((16, MP), F32)
        gw = gw_ref[...].astype(F32).reshape(1, M)
        @pl.loop(0, S // CH)
        def _(c):
            r0 = pl.multiple_of(c * CH, CH)
            xcp(c, r0).wait()
            xf = xt_ref[:, pl.ds(r0, CH)].astype(F32).T
            xc = xf.astype(BF16)
            x_ref[pl.ds(r0, CH), :] = xc
            gl = jnp.sum(xf * gw, axis=-1, keepdims=True)
            g_ref[pl.ds(r0, CH), :] = jax.nn.sigmoid(jnp.broadcast_to(gl, (CH, 128)))
            qkv = _nt(xc, wp_s[:, 0:M])
            qa_s[pl.ds(r0, CH), :] = qkv[:, :MP]
            ka_s[pl.ds(r0 + 16, CH), :] = qkv[:, MP:2 * MP]
            va_s[pl.ds(r0 + 16, CH), :] = qkv[:, 2 * MP:]
        ocp.wait()
        for t in range(5):
            cw = min(128, M - t * 128)
            wt_s[t, 0:M, 0:cw] = wo_ref[:, t * 128:t * 128 + cw].astype(F32)
        for d in range(DH):
            for t in range(5):
                wop_s[d * 32:d * 32 + 32, t * 128:t * 128 + 128] = wt_s[t, pl.ds(d, 32, stride=DH), :]
        wop_s[M:MP, :] = jnp.zeros((MP - M, MP), F32)
        wopt_s[...] = wop_s[...].T[0:M, :].astype(BF16)
        acc_ref[...] = jnp.zeros(acc_ref.shape, F32)
        for c in copies:
            c.wait()

    def local_attn(n):
        r0 = pl.multiple_of(j * AC + n * SC, SC)
        q = qa_s[pl.ds(r0, SC), :]
        kk = ka_s[pl.ds(r0, SC + 16), :]
        vv = va_s[pl.ds(r0, SC + 16), :]
        row = r0 + jax.lax.broadcasted_iota(jnp.int32, (SC, 128), 0)
        lg = []
        for w in range(8):
            pr = q * kk[16 - 2 * w:16 - 2 * w + SC, :]
            t = pr[:, 0:128] + pr[:, 128:256] + pr[:, 256:384] + pr[:, 384:512] + pr[:, 512:640]
            t = t + pltpu.roll(t, 64, 1)
            t = (t + pltpu.roll(t, 32, 1)) * (DH ** -0.5 * LOG2E)
            if w > 0:
                t = jnp.where(row >= 2 * w, t, -1e9)
            lg.append(t)
        m = functools.reduce(jnp.maximum, lg)
        e = [jnp.exp2(t - m) for t in lg]
        inv = g_ref[pl.ds(r0, SC), :] * _recip(functools.reduce(jnp.add, e))
        o = None
        for w in range(8):
            t = jnp.concatenate([e[w] * inv] * 5, axis=1) * vv[16 - 2 * w:16 - 2 * w + SC, :]
            o = t if o is None else o + t
        return o.astype(BF16)

    wq = _pair(wq_s, j, M)
    wk = _pair(wk_s, j, DC)
    wv = _pair(wv_s, j, DC)

    def proj(r0, r1):
        for dst, val in ((q_s, _nn(x_ref[r0:r1, :], wq) * (D ** -0.5 * LOG2E)),
                         (k_s, _nn(c_ref[r0:r1, :], wk)), (v_s, _nn(c_ref[r0:r1, :], wv))):
            if dst is k_s:
                vt = val.T.astype(BF16)
                dst[0, :, r0:r1] = vt[:D]
                dst[1, :, r0:r1] = vt[D:]
                continue
            val = val.astype(BF16)
            dst[0, r0:r1, :] = val[:, :D]
            dst[1, r0:r1, :] = val[:, D:]

    loc = []
    for n in range(4):
        loc.append(local_attn(n))
        proj(n * 512, n * 512 + 512)
    a_s[j] = _nt(wopt_s[...], jnp.concatenate(loc, axis=0))

    @pl.loop(0, 2)
    def _(hh):
        tri = (jax.lax.broadcasted_iota(jnp.int32, (BQ, BQ), 1) <= jax.lax.broadcasted_iota(jnp.int32, (BQ, BQ), 0))
        def score(i, c):
            if c == i:
                r0, h = i * BQ, BQ // 2
                left = _nn(q_s[hh, r0:r0 + BQ, :], k_s[hh, :, r0:r0 + h])
                rb = _nn(q_s[hh, r0 + h:r0 + BQ, :], k_s[hh, :, r0 + h:r0 + BQ])
                right = jnp.concatenate([jnp.full((h, h), -1e9, F32), rb], axis=0)
                return jnp.where(tri, jnp.concatenate([left, right], axis=1), -1e9)
            s = _nn(q_s[hh, i * BQ:(i + 1) * BQ, :], k_s[hh, :, c * BQ:(c + 1) * BQ])
            return s
        fold = lambda op, t: op(t[:, :128], t[:, 128:])
        nxt = [score(NQ - 1, c) for c in range(NQ)]
        mx = functools.reduce(jnp.maximum, [fold(jnp.maximum, s) for s in nxt])
        for i in reversed(range(NQ)):
            r0, r1 = i * BQ, (i + 1) * BQ
            cur, nxt = nxt, []
            m = jnp.broadcast_to(jnp.max(mx, axis=-1, keepdims=True), (BQ, BQ))
            def ahead(c):
                nonlocal mx
                if c < i:
                    s = score(i - 1, c)
                    nxt.append(s)
                    t = fold(jnp.maximum, s)
                    mx = t if c == 0 else jnp.maximum(mx, t)
            ahead(0)
            ctx = l = None
            for c in range(i + 1):
                p = jnp.exp2(cur[c] - m)
                ahead(c + 1)
                t = fold(jnp.add, p)
                l = t if l is None else l + t
                if c == i:
                    h = BQ // 2
                    t = _nn(p[:, :h].astype(BF16), v_s[hh, r0:r0 + h, :])
                    t = jnp.concatenate([t[:h], t[h:] + _nn(p[h:, h:].astype(BF16), v_s[hh, r0 + h:r1, :])], axis=0)
                else:
                    t = _nn(p.astype(BF16), v_s[hh, c * BQ:(c + 1) * BQ, :])
                ctx = t if ctx is None else ctx + t
            l = jnp.sum(l, axis=-1, keepdims=True)
            ctx = (ctx * ((1.0 - g_ref[r0:r1, :]) * _recip(l))).astype(BF16)
            ctx_s[hh, r0:r1, :] = ctx

    wob = jnp.concatenate([wob_ref[0], wob_ref[1]], axis=1)
    for i in range(NQ):
        acc_ref[i] += _nt(wob, jnp.concatenate([ctx_s[0, i * BQ:(i + 1) * BQ, :], ctx_s[1, i * BQ:(i + 1) * BQ, :]], axis=1))

    @pl.when(j == STEPS - 1)
    def _():
        outs = []
        for i in range(NQ):
            cs = slice(i * BQ, (i + 1) * BQ)
            a = jnp.concatenate([a_s[2 * i], a_s[2 * i + 1]], axis=1)
            xt_ref[:, cs] = (acc_ref[i] + a).astype(BF16)
            outs.append(pltpu.make_async_copy(xt_ref.at[:, cs], o_hbm.at[:, cs], sems.at[i]))
            outs[-1].start()
        for c in outs:
            c.wait()


@jax.jit
def pallas_gated_mix__sliding_local_dilated__compressed_kv_cla__prompt_kernel(
    A_x, A_wqkv, A_wo, B_x, B_c_kv, B_w_q, B_w_uk, B_w_uv, B_w_o, gate_w,
):
    del B_x
    hbm = pl.BlockSpec(memory_space=pl.ANY)
    V = pltpu.VMEM
    out = pl.pallas_call(
        _kernel,
        grid=(STEPS,),
        in_specs=[
            hbm, hbm, hbm, hbm, hbm, hbm, hbm,
            pl.BlockSpec((2, M, D), lambda j: (j, 0, 0)),
            pl.BlockSpec((M,), lambda j: (0,)),
        ],
        out_specs=hbm,
        out_shape=jax.ShapeDtypeStruct((M, S), BF16),
        scratch_shapes=[
            V((NQ, M, BQ), F32), V((STEPS, M, AC), F32), V((S, 128), F32),
            V((2, S, D), BF16), V((2, D, S), BF16), V((2, S, D), BF16), V((2, S, D), BF16),
            V((5, 3 * M, 128), F32), V((3 * MP, MP), BF16), V((MP, MP), F32), V((M, MP), BF16),
            V((S, MP), F32), V((S + 16, MP), F32), V((S + 16, MP), F32),
            V((S, M), BF16), V((S, DC), BF16),
            V((M * STEPS, D), U32), V((DC * STEPS, D), U32), V((DC * STEPS, D), U32),
            V((M, S), BF16), V((M, 3 * M), BF16), V((M, M), BF16),
            pltpu.SemaphoreType.DMA((10 + S // CH,)),
        ],
        compiler_params=pltpu.CompilerParams(dimension_semantics=("arbitrary",), vmem_limit_bytes=110 * 1024 * 1024),
    )(A_x.reshape(S, M).T, A_wqkv, A_wo, B_c_kv.reshape(S, DC), B_w_q.reshape(M * H, D),
      B_w_uk.reshape(DC * H, D), B_w_uv.reshape(DC * H, D), B_w_o.transpose(0, 2, 1), gate_w)
    return out.T.reshape(1, S, M)
```
